```python
import jax
import jax.numpy as jnp

def _softmax(x, axis=-1):
    return jax.nn.softmax(x, axis=axis)

def _gelu(x):
    return jax.nn.gelu(x, approximate=True)

def _silu(x):
    return jax.nn.silu(x)

def _sigmoid(x):
    return jax.nn.sigmoid(x)

def _layernorm(x, axis=-1, eps=1e-05):
    m = jnp.mean(x, axis=axis, keepdims=True)
    v = jnp.var(x, axis=axis, keepdims=True)
    return (x - m) / jnp.sqrt(v + eps)

def _scatter_add(tgt, idx, src, axis=0):
    return tgt.at[idx].add(src)

def _segment_sum(src, seg, n):
    return jax.ops.segment_sum(src, seg, n)

class _Rng:

    def __init__(self, key):
        self._k = key

    def _next(self):
        self._k, sub = jax.random.split(self._k)
        return sub

    def normal(self, shape):
        return jax.random.normal(self._next(), shape, dtype=jnp.bfloat16)

    def randint(self, lo, hi, shape):
        return jax.random.randint(self._next(), shape, lo, hi, dtype=jnp.int32)

    def uniform(self, shape, lo=0.0, hi=1.0):
        return jax.random.uniform(self._next(), shape, jnp.bfloat16, lo, hi)

    def permutation(self, n):
        return jax.random.permutation(self._next(), n)
kernel_name = 'interleave_layers__linear_kernel_hedgehog__mixer_gmlp__prompt'

def _fwd_setup_inputs():
    _rng = _Rng(jax.random.key(int.from_bytes(__import__("os").urandom(4), "little")))
    _w = lambda a: (lambda t: t.astype(jnp.bfloat16) if jnp.issubdtype(t.dtype, jnp.floating) else t)(jnp.asarray(a))

    def _A_setup():
        B, S, D, H = (1, 2048, 640, 32)
        Dh = D // H
        return {'x': _w((lambda *s: _rng.normal(s) * 0.05)(B, S, D)), 'wqkv': _w((lambda *s: _rng.normal(s) * 0.05)(D, 3 * D)), 'w_phi': _w((lambda *s: _rng.normal(s) * 0.05)(H, Dh, Dh) * Dh ** (-0.5)), 'wo': _w((lambda *s: _rng.normal(s) * 0.05)(D, D))}
    _A_in = _A_setup()

    def _B_setup():
        B, S, D, F = (1, 2048, 640, 1536)
        Fh = F // 2
        return {'x': _w((lambda *s: _rng.normal(s) * 0.05)(B, S, D)), 'w_in': _w((lambda *s: _rng.normal(s) * 0.05)(D, 2 * Fh)), 'w_sp': _w(0.01 * (lambda *s: _rng.normal(s) * 0.05)(S, S)), 'b_sp': _w(1.0 + 0.01 * (lambda *s: _rng.normal(s) * 0.05)(S)), 'w_out': _w((lambda *s: _rng.normal(s) * 0.05)(Fh, D))}
    _B_in = _B_setup()
    return {'A_x': _A_in['x'], 'A_wqkv': _A_in['wqkv'], 'A_w_phi': _A_in['w_phi'], 'A_wo': _A_in['wo'], 'B_x': _B_in['x'], 'B_w_in': _B_in['w_in'], 'B_w_sp': _B_in['w_sp'], 'B_b_sp': _B_in['b_sp'], 'B_w_out': _B_in['w_out']}

def _fwd_reference(A_x, A_wqkv, A_w_phi, A_wo, B_x, B_w_in, B_w_sp, B_b_sp, B_w_out):

    def _A_ref(x, wqkv, w_phi, wo):
        B, S, D = x.shape
        H = 32
        Dh = D // H
        qkv = (lambda x, *d: x.transpose(*d))((x @ wqkv).reshape(B, S, 3, H, Dh), 2, 0, 3, 1, 4)
        q, k, v = (qkv[0], qkv[1], qkv[2])
        pq = jnp.einsum('bhsd,hdf->bhsf', q, w_phi)
        pk = jnp.einsum('bhsd,hdf->bhsf', k, w_phi)
        phi_q = jnp.concatenate([_softmax(pq, axis=-1), _softmax(-pq, axis=-1)], axis=-1)
        phi_k = jnp.concatenate([_softmax(pk, axis=-1), _softmax(-pk, axis=-1)], axis=-1)
        kv = jnp.einsum('bhsf,bhsd->bhfd', phi_k, v)
        z = jnp.einsum('bhsf->bhf', phi_k)
        num = jnp.einsum('bhqf,bhfd->bhqd', phi_q, kv)
        den = jnp.einsum('bhqf,bhf->bhq', phi_q, z)[..., None] + 1e-06
        o = num / den
        return (lambda x, *d: x.transpose(*d))(o, 0, 2, 1, 3).reshape(B, S, D) @ wo

    def _B_ref(x, w_in, w_sp, b_sp, w_out):
        B, S, D = x.shape
        F = w_in.shape[-1]
        Fh = F // 2
        z = _gelu(jnp.einsum('bsd,df->bsf', x, w_in))
        z1 = z[..., :Fh].copy()
        z2 = _layernorm(z[..., Fh:], axis=-1)
        g = jnp.einsum('ts,bsf->btf', w_sp, z2) + b_sp[None, :, None]
        return jnp.einsum('bsf,fd->bsd', z1 * g, w_out)
    x = A_x
    x = x + _A_ref(_layernorm(x, axis=-1), A_wqkv, A_w_phi, A_wo)
    x = x + _B_ref(_layernorm(x, axis=-1), B_w_in, B_w_sp, B_b_sp, B_w_out)
    x = x + _A_ref(_layernorm(x, axis=-1), A_wqkv, A_w_phi, A_wo)
    x = x + _B_ref(_layernorm(x, axis=-1), B_w_in, B_w_sp, B_b_sp, B_w_out)
    return x

def setup_inputs():
    _inp = _fwd_setup_inputs()
    _gk = jax.random.fold_in(jax.random.key(int.from_bytes(__import__("os").urandom(4), "little")), 2 ** 31 - 1)
    _shapes = [[1, 2048, 640]]
    _dtypes = ['bfloat16']
    _gks = jax.random.split(_gk, len(_shapes))
    _gs = [jax.random.normal(k, s, dtype=jnp.dtype(d)) * 0.05 for k, s, d in zip(_gks, _shapes, _dtypes)]
    _inp['grad_out'] = _gs[0]
    return _inp

def reference(A_x, A_wqkv, A_w_phi, A_wo, B_w_in, B_w_sp, B_b_sp, B_w_out, B_x, grad_out):
    _const = dict(B_x=B_x)

    def _f(*_d):
        return _fwd_reference(**{'A_x': _d[0], 'A_wqkv': _d[1], 'A_w_phi': _d[2], 'A_wo': _d[3], 'B_w_in': _d[4], 'B_w_sp': _d[5], 'B_b_sp': _d[6], 'B_w_out': _d[7], **_const})
    _out, _vjp = jax.vjp(_f, A_x, A_wqkv, A_w_phi, A_wo, B_w_in, B_w_sp, B_b_sp, B_w_out)
    _grads = _vjp(grad_out)
    _out0 = jnp.asarray(_out)
    return (_out0, *[jnp.asarray(_g) for _g in _grads])
```

```python
import math

import jax
import jax.numpy as jnp
import jax.experimental.pallas as pl
import jax.experimental.pallas.tpu as pltpu
from jax import lax

S, D, H, DH, FH = 2048, 640, 32, 20, 768
F2 = 2 * FH
NG, GR = 4, 160
GE = GR + 16
TS = 512
NT = S // TS
T2, T3, T6, T7 = (2048, 1), (512, 1), (256, 1), (256, 1)
BF, F32 = jnp.bfloat16, jnp.float32
C0 = math.sqrt(2.0 / math.pi)
C1 = 0.044715


def _nn(a, b):
    return lax.dot_general(a, b, (((1,), (0,)), ((), ())), preferred_element_type=F32)


def _nt(a, b):
    return lax.dot_general(a, b, (((1,), (1,)), ((), ())), preferred_element_type=F32)


def _tr(a):
    return a.astype(F32).T.astype(BF)


def _ln(x):
    n = x.shape[0]
    m = jnp.sum(x, axis=0, keepdims=True) * (1.0 / n)
    xc = x - m
    v = jnp.sum(xc * xc, axis=0, keepdims=True) * (1.0 / n)
    r = lax.rsqrt(v + 1e-5)
    return xc * r, r


def _ln_bwd(dy, xh, r):
    n = dy.shape[0]
    a = jnp.sum(dy, axis=0, keepdims=True) * (1.0 / n)
    b = jnp.sum(dy * xh, axis=0, keepdims=True) * (1.0 / n)
    return (dy - a - xh * b) * r


def _gelu(x):
    t = jnp.tanh(C0 * (x + C1 * x * x * x))
    return 0.5 * x * (1.0 + t)


def _gelu_grad(x):
    x2 = x * x
    t = jnp.tanh(C0 * (x + C1 * x2 * x))
    hp = 0.5 * (1.0 + t)
    return x * hp, hp + (0.5 * C0) * x * (1.0 - t * t) * (1.0 + (3.0 * C1) * x2)


def _phi(p):
    p3 = p.reshape(DH, 8, p.shape[1])
    ep = jnp.exp(p3 - jnp.max(p3, axis=0, keepdims=True))
    en = jnp.exp(jnp.min(p3, axis=0, keepdims=True) - p3)
    fp = ep * (1.0 / jnp.sum(ep, axis=0, keepdims=True))
    fn = en * (1.0 / jnp.sum(en, axis=0, keepdims=True))
    return fp, fn


def _phi_cat(fp, fn):
    t = fp.shape[2]
    return jnp.concatenate([fp.reshape(GR, t), fn.reshape(GR, t)], axis=0).astype(BF)


def _phi_bwd(fp, fn, dphi):
    t = dphi.shape[1]
    a = dphi[:GR].reshape(DH, 8, t)
    b = dphi[GR:].reshape(DH, 8, t)
    fa = fp * a
    fb = fn * b
    sa = jnp.sum(fa, axis=0, keepdims=True)
    sb = jnp.sum(fb, axis=0, keepdims=True)
    return ((fa - fp * sa) - (fb - fn * sb)).reshape(GR, t)


def _iota2(shape, d):
    return lax.broadcasted_iota(jnp.int32, shape, d)


def _kernel(x_h, wqkv_h, wphi_ref, wo_h, win_h, wsp_h, bsp_ref, wout_h, go_h,
            out_h, dx_h, dwqkv_h, dwphi_ref, dwo_h, dwin_h, dwsp_h, dbsp_ref, dwout_h,
            xin, wqkv, wqkvT, WpT, Wp, wo, wop, wopT, win, winT, wout, woutT, wsp,
            Lm, X, XA, RS, P, O, RD, KV, KVm, KVmT, XB, Hs, Z2, G,
            aW, aWo, aWin, aWout, ost, sst, sem_in, sem_x, sem_o, sem_s, sem_f):
    def cp(src, dst, sem):
        return pltpu.make_async_copy(src, dst, sem)

    def x_copy(src, t):
        r = pl.ds(pl.multiple_of(t * TS, TS), TS)
        return cp(src.at[r, :], xin.at[r, :], sem_x.at[t])

    c_wqkv = cp(wqkv_h, wqkv, sem_in.at[0])
    c_wo = cp(wo_h, wo, sem_in.at[1])
    c_win = cp(win_h, win, sem_in.at[2])
    c_wout = cp(wout_h, wout, sem_in.at[3])
    c_wsp = cp(wsp_h, wsp, sem_in.at[4])
    c_wqkv.start()
    for t in range(NT):
        x_copy(x_h, t).start()
    c_wo.start()
    c_win.start()
    c_wout.start()
    c_wsp.start()

    cur = [TS]

    def lanes(t):
        return pl.ds(pl.multiple_of(t * cur[0], cur[0]), cur[0])

    r160, c160 = _iota2((GR, GR), 0), _iota2((GR, GR), 1)
    pmT = jnp.where((r160 // DH == c160 % 8) & (r160 % DH == c160 // 8), 1.0, 0.0).astype(BF)
    pm = jnp.where((c160 // DH == r160 % 8) & (c160 % DH == r160 // 8), 1.0, 0.0).astype(BF)
    e_fe = jnp.where(_iota2((DH, GR), 0) == _iota2((DH, GR), 1) // 8, 1.0, 0.0).astype(BF)
    hmask = r160 // DH == c160 % 8
    for g in range(NG):
        lt = jnp.where(hmask, _nn(wphi_ref[g * GR:(g + 1) * GR, :], e_fe), 0.0)
        Lm[0, g] = lt.astype(BF)
        Lm[1, g] = lt.T.astype(BF)
    kvmask = _iota2((GE, 2 * GR), 0) % 8 == _iota2((GE, 2 * GR), 1) % 8
    kvmask = kvmask & (_iota2((GE, 2 * GR), 0) < GR + 8)
    def ext_():
        return jnp.where(_iota2((16, cur[0]), 0) < 8, 1.0, 0.0).astype(BF)

    aW[...] = jnp.zeros_like(aW)
    aWo[...] = jnp.zeros_like(aWo)
    aWin[...] = jnp.zeros_like(aWin)
    aWout[...] = jnp.zeros_like(aWout)
    KV[...] = jnp.zeros_like(KV)

    c_wqkv.wait()
    for j in range(3):
        wqkvT[j * D:(j + 1) * D, :] = _tr(wqkv[:, j * D:(j + 1) * D])
    for j in range(3):
        for g in range(NG):
            r = slice(j * D + g * GR, j * D + (g + 1) * GR)
            l = pm if j == 2 else Lm[1, g]
            WpT[r, :] = _nn(l, wqkvT[r, :]).astype(BF)
        Wp[:, j * D:(j + 1) * D] = _tr(WpT[j * D:(j + 1) * D, :])

    def a_fwd1(l, t, x):
        c = lanes(t)
        xh, r = _ln(x)
        xh = xh.astype(BF)
        XA[l, :, c] = xh
        RS[l, :, c] = r
        p = _nn(WpT[D:, :], xh).astype(BF)
        P[l, D:, c] = p
        for g in range(NG):
            fp, fn = _phi(p[g * GR:(g + 1) * GR].astype(F32))
            ve = jnp.concatenate([p[D + g * GR:D + (g + 1) * GR], ext_()], axis=0)
            KV[l, g] += _nt(ve, _phi_cat(fp, fn))
        P[l, :D, c] = _nn(WpT[:D, :], xh).astype(BF)

    def kv_mask(l):
        for g in range(NG):
            m = jnp.where(kvmask, KV[l, g], 0.0)
            KVm[g] = m.astype(BF)
            KVmT[g] = m.T.astype(BF)

    def a_fwd2(l, t, x):
        c = lanes(t)
        os_ = []
        for g in range(NG):
            fp, fn = _phi(P[l, g * GR:(g + 1) * GR, c].astype(F32))
            nd = _nn(KVm[g], _phi_cat(fp, fn))
            rd = 1.0 / (nd[GR:GR + 8] + 1e-6)
            RD[l, g * 8:(g + 1) * 8, c] = rd
            os_.append((nd[:GR].reshape(DH, 8, cur[0]) * rd[None]).reshape(GR, cur[0]).astype(BF))
        o = jnp.concatenate(os_, axis=0)
        O[l, :, c] = o
        return x + _nn(wopT[...], o)

    def b_fwd1(l, t, x):
        c = lanes(t)
        xh, r = _ln(x)
        xh = xh.astype(BF)
        XB[l, :, c] = xh
        RS[2 + l, :, c] = r
        h = _nn(winT[FH:, :], xh).astype(BF)
        Hs[l, FH:, c] = h
        z2, r2 = _ln(_gelu(h.astype(F32)))
        Z2[l * FH:(l + 1) * FH, c] = z2.astype(BF)
        RS[4 + l, :, c] = r2
        h = _nn(winT[:FH, :], xh).astype(BF)
        Hs[l, :FH, c] = h
        G[l, :, c] = _gelu(h.astype(F32)).astype(BF)

    def b_fwd2(l, t, x):
        c = lanes(t)
        g = _nt(Z2[l * FH:(l + 1) * FH, :], wsp[c, :]) + bsp_ref[:, c].astype(F32)
        u = (G[l, :, c].astype(F32) * g).astype(BF)
        G[l, :, c] = g.astype(BF)
        return x + _nn(woutT[...], u)

    def b_bwd1(l, t, dy):
        c = lanes(t)
        dyb = dy.astype(BF)
        du = _nn(wout[...], dyb)
        z1, gp = _gelu_grad(Hs[l, :FH, c].astype(F32))
        g = G[l, :, c].astype(F32)
        dg = du * z1
        G[l, :, c] = dg.astype(BF)
        sdg = jnp.sum(dg, axis=0, keepdims=True)
        if l == 1:
            RS[6, :, c] = sdg
        else:
            dbsp_ref[:, c] = (RS[6, :, c] + sdg).astype(BF)
        Hs[l, :FH, c] = (du * g * gp).astype(BF)
        aWout[...] += _nt((z1 * g).astype(BF), dyb)

    def b_bwd2(l, t, dy):
        c = lanes(t)
        dz2 = _nn(G[l], wsp[:, c])
        z2 = Z2[l * FH:(l + 1) * FH, c].astype(F32)
        _, gp = _gelu_grad(Hs[l, FH:, c].astype(F32))
        dh2 = (_ln_bwd(dz2, z2, RS[4 + l, :, c]) * gp).astype(BF)
        dh = jnp.concatenate([Hs[l, :FH, c], dh2], axis=0)
        xh = XB[l, :, c]
        dxh = _nn(win[...], dh)

        def sink(g):
            q = slice(g * 384, (g + 1) * 384)
            aWin[:, q] += _nt(xh, dh[q])
        return dy + _ln_bwd(dxh, xh.astype(F32), RS[2 + l, :, c]), sink

    def a_bwd1(l, t, dy, sink):
        c = lanes(t)
        dyb = dy.astype(BF)
        do = _nn(wop[...], dyb)
        o = O[l, :, c]
        for g in range(NG):
            sink(g)
            rd = RD[l, g * 8:(g + 1) * 8, c]
            dn = do[g * GR:(g + 1) * GR].reshape(DH, 8, cur[0]) * rd[None]
            og = o[g * GR:(g + 1) * GR].astype(F32).reshape(DH, 8, cur[0])
            dd = -jnp.sum(dn * og, axis=0)
            dne = jnp.concatenate([dn.reshape(GR, cur[0]), dd, jnp.zeros((8, cur[0]), F32)], axis=0).astype(BF)
            fp, fn = _phi(P[l, g * GR:(g + 1) * GR, c].astype(F32))
            KV[l, g] += _nt(dne, _phi_cat(fp, fn))
            dphi = _nn(KVmT[g], dne)
            P[l, g * GR:(g + 1) * GR, c] = _phi_bwd(fp, fn, dphi).astype(BF)
        aWo[...] += _nt(o, dyb)

    def a_bwd2(l, t, dy):
        c = lanes(t)
        xh = XA[l, :, c]
        for g in range(NG):
            rk = slice(D + g * GR, D + (g + 1) * GR)
            rv = slice(2 * D + g * GR, 2 * D + (g + 1) * GR)
            fp, fn = _phi(P[l, rk, c].astype(F32))
            ve = jnp.concatenate([P[l, rv, c], ext_()], axis=0)
            dphi = _nn(KVmT[g], ve)
            P[l, rv, c] = _nn(KVm[g, :GR, :], _phi_cat(fp, fn)).astype(BF)
            P[l, rk, c] = _phi_bwd(fp, fn, dphi).astype(BF)
        dp = P[l, :, c]
        dxh = _nn(Wp[...], dp)

        def sink():
            aW[...] += _nt(dp, xh)
        return dy + _ln_bwd(dxh, xh.astype(F32), RS[l, :, c]), sink

    def load_t(t):
        return xin[lanes(t), :].astype(F32).T

    def o_copy(dst, t):
        return cp(ost.at[lanes(t), :], dst.at[lanes(t), :], sem_o.at[t])

    def emit(dst, t, val):
        ost[lanes(t), :] = val.T.astype(BF)
        o_copy(dst, t).start()

    def loop(f, ts=TS, U=1):
        def body(t, carry):
            f(t)
            return carry
        cur[0] = ts
        lax.fori_loop(0, S // ts, body, 0, unroll=U)
        cur[0] = TS

    def p1(t):
        x_copy(x_h, t).wait()
        x = load_t(t)
        X[:, lanes(t)] = x
        a_fwd1(0, t, x)
    loop(p1)
    for t in range(NT):
        x_copy(go_h, t).start()

    c_wo.wait()
    for g in range(NG):
        wop[g * GR:(g + 1) * GR, :] = _nn(pm, wo[g * GR:(g + 1) * GR, :]).astype(BF)
    wopT[...] = _tr(wop[...])
    c_win.wait()
    winT[...] = _tr(win[...])

    def p2(l):
        def f(t):
            x = a_fwd2(l, t, X[:, lanes(t)])
            X[:, lanes(t)] = x
            b_fwd1(l, t, x)
        kv_mask(l)
        loop(f, *T2)

    p2(0)
    c_wout.wait()
    woutT[...] = _tr(wout[...])
    c_wsp.wait()

    def p3(t):
        x = b_fwd2(0, t, X[:, lanes(t)])
        X[:, lanes(t)] = x
        a_fwd1(1, t, x)
    loop(p3, *T3)
    p2(1)

    def p5(t):
        x = b_fwd2(1, t, X[:, lanes(t)])
        emit(out_h, t, x)
        x_copy(go_h, t).wait()
        dy = load_t(t)
        X[:, lanes(t)] = dy
        b_bwd1(1, t, dy)
    loop(p5)

    def p6(l):
        kv_mask(l)
        KV[l] = jnp.zeros_like(KV[l])

        def f(t):
            dy, sink = b_bwd2(l, t, X[:, lanes(t)])
            X[:, lanes(t)] = dy
            a_bwd1(l, t, dy, sink)
        loop(f, *T6)
        kv_mask(l)

    p6(1)

    def p7(t):
        dy, sink = a_bwd2(1, t, X[:, lanes(t)])
        X[:, lanes(t)] = dy
        sink()
        b_bwd1(0, t, dy)
    loop(p7, *T7)
    for t in range(NT):
        o_copy(out_h, t).wait()

    wout[...] = aWout[...].astype(BF)
    f_wout = cp(wout, dwout_h, sem_f.at[0])
    f_wout.start()

    def s_copy(t):
        return cp(sst.at[t], dwsp_h.at[lanes(t), :], sem_s.at[t])

    def psp(t):
        c = lanes(t)
        dgt = jnp.concatenate([_tr(G[0, :, c]), _tr(G[1, :, c])], axis=1)
        sst[t] = _nn(dgt, Z2[...]).astype(BF)
        s_copy(t).start()
    loop(psp)

    p6(0)
    win[...] = aWin[...].astype(BF)
    f_win = cp(win, dwin_h, sem_f.at[1])
    f_win.start()
    for g in range(NG):
        r = slice(g * GR, (g + 1) * GR)
        wo[r, :] = _nn(pmT, aWo[r, :].astype(BF)).astype(BF)
    f_wo = cp(wo, dwo_h, sem_f.at[2])
    f_wo.start()

    def p9(t):
        dy, sink = a_bwd2(0, t, X[:, lanes(t)])
        emit(dx_h, t, dy)
        sink()
    loop(p9)

    dl = [jnp.zeros((GR, GR), F32) for _ in range(NG)]
    for j in range(3):
        for g in range(NG):
            r = slice(j * D + g * GR, j * D + (g + 1) * GR)
            a = aW[r, :].astype(BF)
            lt = pmT if j == 2 else Lm[0, g]
            WpT[r, :] = _nn(lt, a).astype(BF)
            if j < 2:
                dl[g] = dl[g] + _nt(wqkvT[r, :], a)
        wqkv[:, j * D:(j + 1) * D] = _tr(WpT[j * D:(j + 1) * D, :])
    f_wqkv = cp(wqkv, dwqkv_h, sem_f.at[3])
    f_wqkv.start()
    for g in range(NG):
        m = jnp.where(hmask, dl[g], 0.0).astype(BF)
        dwphi_ref[g * GR:(g + 1) * GR, :] = _nt(m, e_fe).astype(BF)

    for t in range(NT):
        o_copy(dx_h, t).wait()
        s_copy(t).wait()
    f_wout.wait()
    f_win.wait()
    f_wo.wait()
    f_wqkv.wait()


@jax.jit
def pallas_interleave_layers__linear_kernel_hedgehog__mixer_gmlp__prompt_kernel(
    A_x, A_wqkv, A_w_phi, A_wo, B_x, B_w_in, B_w_sp, B_b_sp, B_w_out, grad_out,
):
    del B_x
    hbm = pl.BlockSpec(memory_space=pl.ANY)
    vm = pl.BlockSpec(memory_space=pltpu.VMEM)
    sd = jax.ShapeDtypeStruct
    V = pltpu.VMEM
    scratch = [
        V((S, D), BF),
        V((D, 3 * D), BF),
        V((3 * D, D), BF),
        V((3 * D, D), BF),
        V((D, 3 * D), BF),
        V((D, D), BF), V((D, D), BF), V((D, D), BF),
        V((D, F2), BF), V((F2, D), BF),
        V((FH, D), BF), V((D, FH), BF),
        V((S, S), BF),
        V((2, NG, GR, GR), BF),
        V((D, S), F32),
        V((2, D, S), BF),
        V((7, 1, S), F32),
        V((2, 3 * D, S), BF),
        V((2, D, S), BF),
        V((2, H, S), F32),
        V((2, NG, GE, 2 * GR), F32),
        V((NG, GE, 2 * GR), BF),
        V((NG, 2 * GR, GE), BF),
        V((2, D, S), BF),
        V((2, F2, S), BF),
        V((F2, S), BF),
        V((2, FH, S), BF),
        V((3 * D, D), F32), V((D, D), F32), V((D, F2), F32), V((FH, D), F32),
        V((S, D), BF),
        V((NT, TS, S), BF),
        pltpu.SemaphoreType.DMA((5,)),
        pltpu.SemaphoreType.DMA((NT,)),
        pltpu.SemaphoreType.DMA((NT,)),
        pltpu.SemaphoreType.DMA((NT,)),
        pltpu.SemaphoreType.DMA((4,)),
    ]
    outs = pl.pallas_call(
        _kernel,
        in_specs=[hbm, hbm, vm, hbm, hbm, hbm, vm, hbm, hbm],
        out_specs=[hbm, hbm, hbm, vm, hbm, hbm, hbm, vm, hbm],
        out_shape=[sd((S, D), BF), sd((S, D), BF), sd((D, 3 * D), BF), sd((H * DH, DH), BF),
                   sd((D, D), BF), sd((D, F2), BF), sd((S, S), BF), sd((1, S), BF),
                   sd((FH, D), BF)],
        scratch_shapes=scratch,
        compiler_params=pltpu.CompilerParams(vmem_limit_bytes=126 * 1024 * 1024),
    )(A_x.reshape(S, D), A_wqkv, A_w_phi.reshape(H * DH, DH), A_wo, B_w_in, B_w_sp,
      B_b_sp.reshape(1, S), B_w_out, grad_out.reshape(S, D))
    out, dx, dwqkv, dwphi, dwo, dwin, dwsp, dbsp, dwout = outs
    return (out.reshape(1, S, D), dx.reshape(1, S, D), dwqkv, dwphi.reshape(H, DH, DH),
            dwo, dwin, dwsp, dbsp.reshape(S), dwout)
```
